```python
import jax
import jax.numpy as jnp

def _softmax(x, axis=-1):
    return jax.nn.softmax(x, axis=axis)

def _gelu(x):
    return jax.nn.gelu(x, approximate=True)

def _silu(x):
    return jax.nn.silu(x)

def _sigmoid(x):
    return jax.nn.sigmoid(x)

def _layernorm(x, axis=-1, eps=1e-05):
    m = jnp.mean(x, axis=axis, keepdims=True)
    v = jnp.var(x, axis=axis, keepdims=True)
    return (x - m) / jnp.sqrt(v + eps)

def _scatter_add(tgt, idx, src, axis=0):
    return tgt.at[idx].add(src)

def _segment_sum(src, seg, n):
    return jax.ops.segment_sum(src, seg, n)

class _Rng:

    def __init__(self, key):
        self._k = key

    def _next(self):
        self._k, sub = jax.random.split(self._k)
        return sub

    def normal(self, shape):
        return jax.random.normal(self._next(), shape, dtype=jnp.bfloat16)

    def randint(self, lo, hi, shape):
        return jax.random.randint(self._next(), shape, lo, hi, dtype=jnp.int32)

    def uniform(self, shape, lo=0.0, hi=1.0):
        return jax.random.uniform(self._next(), shape, jnp.bfloat16, lo, hi)

    def permutation(self, n):
        return jax.random.permutation(self._next(), n)
kernel_name = 'adaLN_cond__memory_aug_recurrent_mem_tr__moe_arch_mod__prompt'

def setup_inputs():
    _rng = _Rng(jax.random.key(int.from_bytes(__import__("os").urandom(4), "little")))
    _w = lambda a: (lambda t: t.astype(jnp.bfloat16) if jnp.issubdtype(t.dtype, jnp.floating) else t)(jnp.asarray(a))

    def _A_setup():
        B, S, Dm = (1, 2048, 1024)
        H, Dh = (32, 128)
        M, seg = (8, 32)
        seg = min(seg, S)
        S = S // seg * seg
        return {'x': _w((lambda *s: _rng.normal(s) * 0.05)(B, S, Dm)), 'mem0': _w((lambda *s: _rng.normal(s) * 0.05)(B, M, Dm)), 'Wq': _w((lambda *s: _rng.normal(s) * 0.05)(Dm, H, Dh) * Dm ** (-0.5)), 'Wk': _w((lambda *s: _rng.normal(s) * 0.05)(Dm, H, Dh) * Dm ** (-0.5)), 'Wv': _w((lambda *s: _rng.normal(s) * 0.05)(Dm, H, Dh) * Dm ** (-0.5)), 'Wo': _w((lambda *s: _rng.normal(s) * 0.05)(H, Dh, Dm) * (H * Dh) ** (-0.5)), 'seg_len': seg}
    _A_in = _A_setup()

    def _B_setup():
        B, S, D, F, C = (1, 2048, 1024, 3584, 2)
        return {'x': _w((lambda *s: _rng.normal(s) * 0.05)(B, S, D)), 'w_r': _w((lambda *s: _rng.normal(s) * 0.05)(D)), 'w_gate': _w((lambda *s: _rng.normal(s) * 0.05)(D, F)), 'w_up': _w((lambda *s: _rng.normal(s) * 0.05)(D, F)), 'w_down': _w((lambda *s: _rng.normal(s) * 0.05)(F, D))}
    _B_in = _B_setup()
    return {'A_x': _A_in['x'], 'A_mem0': _A_in['mem0'], 'A_Wq': _A_in['Wq'], 'A_Wk': _A_in['Wk'], 'A_Wv': _A_in['Wv'], 'A_Wo': _A_in['Wo'], 'A_seg_len': _A_in['seg_len'], 'B_x': _B_in['x'], 'B_w_r': _B_in['w_r'], 'B_w_gate': _B_in['w_gate'], 'B_w_up': _B_in['w_up'], 'B_w_down': _B_in['w_down'], 'c': _w((lambda *s: _rng.normal(s) * 0.05)(1, 1024)), 'w_mod': _w((lambda *s: _rng.normal(s) * 0.05)(1024, 6 * 1024) * 1024 ** (-0.5))}

def reference(A_x, A_mem0, A_Wq, A_Wk, A_Wv, A_Wo, A_seg_len, B_x, B_w_r, B_w_gate, B_w_up, B_w_down, c, w_mod):

    def _A_ref(x, mem0, Wq, Wk, Wv, Wo, seg_len):
        B, S, Dm = x.shape
        H, Dh = (Wq.shape[1], Wq.shape[2])
        M = mem0.shape[1]
        scale = Dh ** (-0.5)
        n_seg = S // seg_len
        L = M + seg_len
        idx = jnp.arange(L)
        mask = (idx[:, None] < M) | (idx[:, None] >= idx[None, :])
        mem = mem0
        outs = []
        for s in range(n_seg):
            xs = x[:, s * seg_len:(s + 1) * seg_len, :].copy()
            h = jnp.concatenate([mem, xs], axis=1)
            q = jnp.einsum('btd,dhe->bhte', h, Wq)
            k = jnp.einsum('btd,dhe->bhte', h, Wk)
            v = jnp.einsum('btd,dhe->bhte', h, Wv)
            scores = jnp.einsum('bhqe,bhke->bhqk', q, k) * scale
            scores = jnp.where(mask[None, None], scores, -1000000000.0)
            p = _softmax(scores, axis=-1)
            o = jnp.einsum('bhqk,bhke->bhqe', p, v)
            o = jnp.einsum('bhte,hed->btd', o, Wo)
            mem = o[:, :M, :].copy()
            outs.append(o[:, M:, :])
        return jnp.concatenate(outs, axis=1)

    def _B_ref(x, w_r, w_gate, w_up, w_down):
        B, S, D = x.shape
        C = 2
        r = x @ w_r
        idx = jnp.argsort(-r, axis=-1)[:, :C]
        idx_e = jnp.repeat(idx.reshape(B, C, 1), D, axis=2)
        x_sel = jnp.take_along_axis(x, idx_e, axis=1)
        g = _silu(x_sel @ w_gate)
        u = x_sel @ w_up
        y = g * u @ w_down
        r_sel = _sigmoid(jnp.take_along_axis(r, idx, axis=1))
        y = y * r_sel.reshape(B, C, 1)
        b_off = (jnp.arange(B) * S).reshape(B, 1)
        flat_idx = (idx + b_off).reshape(B * C)
        zero = (x * 0.0).reshape(B * S, D)
        upd = _scatter_add(zero, flat_idx, y.reshape(B * C, D), axis=0)
        return x + upd.reshape(B, S, D)
    x = A_x
    mod = (_silu(c) @ w_mod).reshape(c.shape[0], 6, 1, -1)
    sa, ca, ga, sb, cb, gb = (mod[:, 0].copy(), mod[:, 1].copy(), mod[:, 2].copy(), mod[:, 3].copy(), mod[:, 4].copy(), mod[:, 5].copy())
    h = _layernorm(x, axis=-1) * (1 + ca) + sa
    x = x + ga * _A_ref(h, A_mem0, A_Wq, A_Wk, A_Wv, A_Wo, A_seg_len)
    h = _layernorm(x, axis=-1) * (1 + cb) + sb
    x = x + gb * _B_ref(h, B_w_r, B_w_gate, B_w_up, B_w_down)
    return x
```

```python
import functools
import jax
import jax.numpy as jnp
from jax import lax
import jax.experimental.pallas as pl
import jax.experimental.pallas.tpu as pltpu

F32 = jnp.float32
BF16 = jnp.bfloat16
U32 = jnp.uint32
UNROLL = 1


def _mm(a, b):
    return lax.dot_general(a, b, (((1,), (0,)), ((), ())), preferred_element_type=F32)


def _mm_nt(a, b):
    return lax.dot_general(a, b, (((1,), (1,)), ((), ())), preferred_element_type=F32)


def _ln(x, eps=1e-5):
    m = jnp.mean(x, axis=-1, keepdims=True)
    d = x - m
    v = jnp.mean(d * d, axis=-1, keepdims=True)
    return d * lax.rsqrt(v + eps)


def _rb(x):
    return x.astype(BF16).astype(F32)


def make_kernel(S, D, H, E, M, SEG, FF, G):
    NSEG = S // SEG
    L = M + SEG
    HE = H * E
    DC = 128
    NCH = D // DC
    NSLOT = 4
    PF = NSLOT - 1
    XS0 = 6
    LAG = 2
    scale = float(E) ** -0.5
    HP = H // 2

    def kernel(x_hbm, mem0_ref, wq_hbm, wk_hbm, wv_hbm, wo_hbm, wr_ref, wg_hbm, wu_hbm, wd_hbm,
               c_ref, wmod_hbm, out_hbm,
               wq, wk, wv, wo, wg, wu, wd, wmodA, wmodB, stage, xs, mods, hbuf, obuf, x1s, rbuf, ostage, xsel,
               sem_st, sem_w, sem_o):
        wmod_u = wmod_hbm.bitcast(U32)
        cp_modA = pltpu.make_async_copy(wmod_u.at[:, pl.ds(0, 2 * D)], wmodA, sem_w.at[0])
        cp_modB = pltpu.make_async_copy(wmod_u.at[:, pl.ds(2 * D, 4 * D)], wmodB, sem_w.at[1])
        cp_x0 = pltpu.make_async_copy(x_hbm.at[pl.ds(0, XS0 * SEG)], xs.at[pl.ds(0, XS0 * SEG)], sem_w.at[2])
        cp_x1 = pltpu.make_async_copy(x_hbm.at[pl.ds(XS0 * SEG, S - XS0 * SEG)],
                                      xs.at[pl.ds(XS0 * SEG, S - XS0 * SEG)], sem_w.at[3])
        cp_wo = pltpu.make_async_copy(wo_hbm.bitcast(U32), wo, sem_w.at[4])
        cp_wg = pltpu.make_async_copy(wg_hbm.bitcast(U32), wg, sem_w.at[5])
        cp_wu = pltpu.make_async_copy(wu_hbm.bitcast(U32), wu, sem_w.at[6])
        cp_wd = pltpu.make_async_copy(wd_hbm.bitcast(U32), wd, sem_w.at[7])
        srcs = [wq_hbm.bitcast(U32), wk_hbm.bitcast(U32), wv_hbm.bitcast(U32)]
        dsts = [wq, wk, wv]

        def cp(w, c, slot):
            return pltpu.make_async_copy(srcs[w].at[pl.ds(c * DC * HP, DC * HP)], stage.at[slot], sem_st.at[slot])

        cp_modA.start()
        cp_x0.start()
        for n in range(PF):
            cp(0, n, n).start()

        cc = c_ref[...].astype(F32)
        sc8 = jnp.broadcast_to(cc * jax.nn.sigmoid(cc), (8, D))
        mods[:, 2 * D:6 * D] = jnp.zeros((8, 4 * D), F32)
        cp_modA.wait()
        mods[:, 0:2 * D] = _rb(_mm(sc8, pltpu.bitcast(wmodA[...], BF16)))

        def mod_row(i):
            return mods[0:1, i * D:(i + 1) * D]

        def ln1(seg):
            xv = xs[pl.ds(pl.multiple_of(seg * SEG, SEG), SEG), :].astype(F32)
            return _ln(xv) * (1.0 + mod_row(1)) + mod_row(0)

        cp_x0.wait()
        hbuf[0] = ln1(0)
        for i in range(LAG + 1):
            obuf[i] = jnp.zeros((SEG, D), F32)
        rbuf[...] = jnp.full((SEG, 128), -jnp.inf, F32)

        for w in range(3):
            dst = dsts[w]

            def body(c, carry, dst=dst, w=w):
                n = w * NCH + c
                slot = n % NSLOT
                nslot = (n + PF) % NSLOT
                cp(w, c, slot).wait()

                @pl.when(c + PF < NCH)
                def _():
                    cp(w, c + PF, nslot).start()
                if w < 2:
                    @pl.when(c + PF >= NCH)
                    def _():
                        cp(w + 1, c + PF - NCH, nslot).start()
                else:
                    @pl.when(c + PF == NCH)
                    def _():
                        cp_wo.start()
                for b in range(DC // 16):
                    for j in range(HP):
                        ev = stage[slot, pl.ds((b * 16) * HP + j, 8, stride=H), :]
                        od = stage[slot, pl.ds((b * 16 + 1) * HP + j, 8, stride=H), :]
                        lo = (ev & jnp.uint32(0xFFFF)) | (od << 16)
                        hi = (ev >> 16) | (od & jnp.uint32(0xFFFF0000))
                        r0 = pl.multiple_of(c * (DC // 2) + b * 8, 8)
                        dst[pl.ds(r0, 8), (2 * j) * E:(2 * j + 1) * E] = lo
                        dst[pl.ds(r0, 8), (2 * j + 1) * E:(2 * j + 2) * E] = hi
                return carry
            lax.fori_loop(0, NCH, body, 0)
        cp_wo.wait()
        cp_modB.start()
        cp_x1.start()
        cp_wg.start()
        cp_wu.start()
        cp_wd.start()

        row = lax.broadcasted_iota(jnp.int32, (L, L), 0)
        col = lax.broadcasted_iota(jnp.int32, (L, L), 1)
        mask = (row < M) | (row >= col)
        lane = lax.broadcasted_iota(jnp.int32, (SEG, 128), 1)

        def out_copy(seg):
            r0 = pl.multiple_of(seg * SEG, SEG)
            return pltpu.make_async_copy(ostage.at[pl.ds(r0, SEG)], out_hbm.at[pl.ds(r0, SEG)], sem_o.at[0])

        def epilogue(seg, o, valid):
            r0 = pl.multiple_of(seg * SEG, SEG)
            xv = xs[pl.ds(r0, SEG), :].astype(F32)
            x1 = _rb(xv + mod_row(2) * o)
            x1s[pl.ds(r0, SEG), :] = x1
            h2 = _rb(_ln(x1) * (1.0 + mod_row(4)) + mod_row(3))
            r = _rb(jnp.sum(h2 * wr_ref[...].astype(F32), axis=-1, keepdims=True))
            rbuf[...] = jnp.where(lane == jnp.where(valid, seg, -1), r, rbuf[...])
            ostage[pl.ds(r0, SEG), :] = (x1 + mod_row(5) * h2).astype(BF16)

        def step(s, mem):
            @pl.when(s == LAG)
            def _():
                cp_modB.wait()
                mods[:, 2 * D:6 * D] = _rb(_mm(sc8, pltpu.bitcast(wmodB[...], BF16)))
                cp_x1.wait()

            @pl.when(s > LAG)
            def _():
                out_copy(s - LAG - 1).start()

            cur = s % 2
            nxt = 1 - cur
            hh = jnp.concatenate([mem, hbuf[cur]], axis=0)
            NG = H // G
            st = {}

            def proj(w, g):
                return _mm(hh, pltpu.bitcast(w[:, g * G * E:(g + 1) * G * E], BF16))

            def Q(g):
                st['q', g] = proj(wq, g)

            def K(g):
                st['k', g] = proj(wk, g).astype(BF16)

            def V(g):
                st['v', g] = proj(wv, g).astype(BF16)

            def SC(g):
                q, k = st['q', g], st['k', g]
                st['s', g] = [_mm_nt(q[:, hd * E:(hd + 1) * E], k[:, hd * E:(hd + 1) * E]) for hd in range(G)]

            def PV(g):
                v = st['v', g]
                os_ = []
                for hd in range(G):
                    sc = jnp.where(mask, st['s', g][hd] * scale, -1e9)
                    mx = jnp.max(sc, axis=-1, keepdims=True)
                    e = jnp.exp(sc - mx)
                    p = e / jnp.sum(e, axis=-1, keepdims=True)
                    os_.append(_mm(p, v[:, hd * E:(hd + 1) * E]))
                st['o', g] = jnp.concatenate(os_, axis=1)

            def WO(g):
                part = _mm(st['o', g], pltpu.bitcast(wo[g * G * (E // 2):(g + 1) * G * (E // 2), :], BF16))
                st['acc'] = part if 'acc' not in st else st['acc'] + part

            Q(0); K(0); V(0)
            for g in range(NG - 1):
                SC(g); Q(g + 1); K(g + 1); PV(g); V(g + 1)
                if g >= 2:
                    WO(g - 2)
                if g == 1:
                    hbuf[nxt] = ln1(jnp.minimum(s + 1, NSEG - 1))
                if g == 3:
                    epilogue(jnp.maximum(s - LAG, 0), obuf[(s + 1) % (LAG + 1)], s >= LAG)
            g = NG - 1
            SC(g); WO(g - 2); WO(g - 1); PV(g); WO(g)
            acc = st['acc']
            obuf[s % (LAG + 1)] = acc[M:L]
            return acc[0:M]
        lax.fori_loop(0, NSEG, step, mem0_ref[...].astype(F32), unroll=UNROLL)
        out_copy(NSEG - LAG - 1).start()
        for t in range(NSEG - LAG, NSEG):
            epilogue(t, obuf[t % (LAG + 1)], True)
            out_copy(t).start()

        rv = rbuf[...]
        ridx = lane * SEG + lax.broadcasted_iota(jnp.int32, (SEG, 128), 0)

        def allmax(a):
            return jnp.max(jnp.max(a, axis=1, keepdims=True), axis=0, keepdims=True)

        def allmin(a):
            return jnp.min(jnp.min(a, axis=1, keepdims=True), axis=0, keepdims=True)
        m1 = allmax(rv)
        i1 = allmin(jnp.where(rv == m1, ridx, S))
        rv2 = jnp.where(ridx == i1, -jnp.inf, rv)
        m2 = allmax(rv2)
        i2 = allmin(jnp.where(rv2 == m2, ridx, S))
        i1s = jnp.clip(i1[0, 0], 0, S - 1)
        i2s = jnp.clip(i2[0, 0], 0, S - 1)
        xsel[...] = jnp.zeros((8, D), F32)
        xsel[0:1, :] = x1s[pl.ds(i1s, 1), :]
        xsel[1:2, :] = x1s[pl.ds(i2s, 1), :]
        x1sel = xsel[...]
        h2 = _rb(_ln(x1sel) * (1.0 + mod_row(4)) + mod_row(3))
        cp_wg.wait()
        gte = _rb(_mm(h2, pltpu.bitcast(wg[...], BF16)))
        cp_wu.wait()
        up = _rb(_mm(h2, pltpu.bitcast(wu[...], BF16)))
        act = _rb(gte * jax.nn.sigmoid(gte)) * up
        cp_wd.wait()
        y = _rb(_mm(act, pltpu.bitcast(wd[...], BF16)))
        rid8 = lax.broadcasted_iota(jnp.int32, (8, D), 0)
        rsel = jnp.where(rid8 == 0, jnp.broadcast_to(m1, (8, D)), jnp.broadcast_to(m2, (8, D)))
        y = _rb(y * _rb(jax.nn.sigmoid(rsel)))
        fin = x1sel + _rb(mod_row(5) * _rb(h2 + y))
        pltpu.make_async_copy(ostage, out_hbm, sem_o.at[0]).wait()
        bs = []
        for t, ii in ((0, i1s), (1, i2s)):
            b0 = pl.multiple_of((ii // 16) * 16, 16)
            blk = ostage[pl.ds(b0, 16), :].astype(F32)
            rid = lax.broadcasted_iota(jnp.int32, (16, D), 0) + b0
            new = jnp.where(rid == ii, jnp.broadcast_to(fin[t:t + 1, :], (16, D)), blk)
            ostage[pl.ds(b0, 16), :] = new.astype(BF16)
            bs.append(b0)
        for t in range(2):
            cpo = pltpu.make_async_copy(ostage.at[pl.ds(bs[t], 16)], out_hbm.at[pl.ds(bs[t], 16)], sem_o.at[1])
            cpo.start()
            cpo.wait()

    scratch = [
        pltpu.VMEM((D // 2, HE), U32), pltpu.VMEM((D // 2, HE), U32), pltpu.VMEM((D // 2, HE), U32),
        pltpu.VMEM((HE // 2, D), U32),
        pltpu.VMEM((D // 2, FF), U32), pltpu.VMEM((D // 2, FF), U32), pltpu.VMEM((FF // 2, D), U32),
        pltpu.VMEM((D // 2, 2 * D), U32), pltpu.VMEM((D // 2, 4 * D), U32),
        pltpu.VMEM((NSLOT, DC * HP, E), U32),
        pltpu.VMEM((S, D), BF16),
        pltpu.VMEM((8, 6 * D), F32),
        pltpu.VMEM((2, SEG, D), F32),
        pltpu.VMEM((LAG + 1, SEG, D), F32),
        pltpu.VMEM((S, D), F32),
        pltpu.VMEM((SEG, 128), F32),
        pltpu.VMEM((S, D), BF16),
        pltpu.VMEM((8, D), F32),
        pltpu.SemaphoreType.DMA((NSLOT,)),
        pltpu.SemaphoreType.DMA((8,)),
        pltpu.SemaphoreType.DMA((2,)),
    ]
    return kernel, scratch


@functools.partial(jax.jit, static_argnames=("A_seg_len",))
def pallas_adaLN_cond__memory_aug_recurrent_mem_tr__moe_arch_mod__prompt_kernel(
        A_x, A_mem0, A_Wq, A_Wk, A_Wv, A_Wo, A_seg_len, B_x, B_w_r, B_w_gate, B_w_up, B_w_down, c, w_mod):
    B, S, D = A_x.shape
    _, H, E = A_Wq.shape
    M = A_mem0.shape[1]
    FF = B_w_gate.shape[1]
    assert B == 1
    kernel, scratch = make_kernel(S, D, H, E, M, int(A_seg_len), FF, 4)
    hbm = pl.BlockSpec(memory_space=pl.ANY)
    vm = pl.BlockSpec(memory_space=pltpu.VMEM)
    out = pl.pallas_call(
        kernel,
        out_shape=jax.ShapeDtypeStruct((S, D), A_x.dtype),
        in_specs=[hbm, vm, hbm, hbm, hbm, hbm, vm, hbm, hbm, hbm, vm, hbm],
        out_specs=hbm,
        scratch_shapes=scratch,
        compiler_params=pltpu.CompilerParams(vmem_limit_bytes=120 * 2**20),
    )(A_x.reshape(S, D), A_mem0.reshape(M, D), A_Wq.reshape(D * H, E), A_Wk.reshape(D * H, E),
      A_Wv.reshape(D * H, E), A_Wo.reshape(H * E, D), B_w_r.reshape(1, D), B_w_gate, B_w_up, B_w_down, c, w_mod)
    return out.reshape(B, S, D)
```

```python
import functools
import jax
import jax.numpy as jnp
from jax import lax
import jax.experimental.pallas as pl
import jax.experimental.pallas.tpu as pltpu

F32 = jnp.float32
BF16 = jnp.bfloat16
U32 = jnp.uint32
KPRE = 4


def _mm(a, b):
    return lax.dot_general(a, b, (((1,), (0,)), ((), ())), preferred_element_type=F32)


def _mm_q(a, b):
    return lax.dot_general(a, b, (((1,), (0,)), ((), ())), preferred_element_type=F32)
def _mm_k(a, b):
    return lax.dot_general(a, b, (((1,), (0,)), ((), ())), preferred_element_type=F32)
def _mm_v(a, b):
    return lax.dot_general(a, b, (((1,), (0,)), ((), ())), preferred_element_type=F32)
def _mm_pv(a, b):
    return lax.dot_general(a, b, (((1,), (0,)), ((), ())), preferred_element_type=F32)
def _mm_o(a, b):
    return lax.dot_general(a, b, (((1,), (0,)), ((), ())), preferred_element_type=F32)
def _mm_o2(a, b):
    return lax.dot_general(a, b, (((1,), (0,)), ((), ())), preferred_element_type=F32)


def _mm_nt(a, b):
    return lax.dot_general(a, b, (((1,), (1,)), ((), ())), preferred_element_type=F32)


def _ln(x, eps=1e-5):
    m = jnp.mean(x, axis=-1, keepdims=True)
    d = x - m
    v = jnp.mean(d * d, axis=-1, keepdims=True)
    return d * lax.rsqrt(v + eps)


def _recip(s):
    r = pl.reciprocal(s, approx=True)
    return r * (2.0 - s * r)


def _rb(x):
    return x.astype(BF16).astype(F32)


def make_kernel(S, D, H, E, M, SEG, FF, G):
    NSEG = S // SEG
    L = M + SEG
    HE = H * E
    DC = 128
    NCH = D // DC
    NSLOT = 3
    PF = NSLOT - 1
    PR = 8
    NG = H // G
    GE = G * E
    NKP = KPRE
    XS0 = 6
    LAG = 2
    scale = float(E) ** -0.5
    HP = H // 2

    def kernel(x_hbm, x3_hbm, mem0_ref, wq_hbm, wk_hbm, wv_hbm, wo_hbm, wr_ref, wg_hbm, wu_hbm, wd_hbm,
               c_ref, wmod_hbm, out_hbm,
               wq, wkv, wo, wg, wu, wd, wmodA, wmodB, stage, xs, xpre, hpre, qpre, kpre, mods, hbuf, obuf, x1s, rbuf, ostage, xsel,
               sem_st, sem_w, sem_o):
        wmod_u = wmod_hbm.bitcast(U32)
        cp_modA = pltpu.make_async_copy(wmod_u.at[:, pl.ds(0, 2 * D)], wmodA, sem_w.at[0])
        cp_modB = pltpu.make_async_copy(wmod_u.at[:, pl.ds(2 * D, 4 * D)], wmodB, sem_w.at[1])
        cp_x0 = pltpu.make_async_copy(x_hbm.at[pl.ds(0, XS0 * SEG)], xs.at[pl.ds(0, XS0 * SEG)], sem_w.at[2])
        cp_x1 = pltpu.make_async_copy(x_hbm.at[pl.ds(XS0 * SEG, S - XS0 * SEG)],
                                      xs.at[pl.ds(XS0 * SEG, S - XS0 * SEG)], sem_w.at[3])
        cp_wo = pltpu.make_async_copy(wo_hbm.bitcast(U32), wo, sem_w.at[4])
        cp_wg = pltpu.make_async_copy(wg_hbm.bitcast(U32), wg, sem_w.at[5])
        cp_wu = pltpu.make_async_copy(wu_hbm.bitcast(U32), wu, sem_w.at[6])
        cp_wd = pltpu.make_async_copy(wd_hbm.bitcast(U32), wd, sem_w.at[7])
        srcs = [wq_hbm.bitcast(U32), wk_hbm.bitcast(U32), wv_hbm.bitcast(U32)]
        cp_xp = pltpu.make_async_copy(x3_hbm.at[:, pl.ds(SEG - PR, PR), :], xpre, sem_w.at[8])

        def cp(w, c, slot):
            return pltpu.make_async_copy(srcs[w].at[pl.ds(c * 2 * DC * HP, 2 * DC * HP)], stage.at[slot], sem_st.at[slot])

        cp_modA.start()
        cp_xp.start()
        cp_x0.start()
        for n in range(PF):
            cp(0, n, n).start()

        cc = c_ref[...].astype(F32)
        sc8 = jnp.broadcast_to(cc * jax.nn.sigmoid(cc), (8, D))
        mods[:, 2 * D:6 * D] = jnp.zeros((8, 4 * D), F32)
        cp_modA.wait()
        mods[:, 0:2 * D] = _rb(_mm(sc8, pltpu.bitcast(wmodA[...], BF16)))

        def mod_row(i):
            return mods[0:1, i * D:(i + 1) * D]

        def ln1(seg):
            xv = xs[pl.ds(pl.multiple_of(seg * SEG, SEG), SEG), :].astype(F32)
            return _ln(xv) * (1.0 + mod_row(1)) + mod_row(0)

        cp_xp.wait()
        xp = xpre[...].astype(F32).reshape(NSEG * PR, D)
        hpre[...] = _ln(xp) * (1.0 + mod_row(1)) + mod_row(0)
        cp_x0.wait()
        hbuf[0] = ln1(0)
        for i in range(4):
            obuf[i] = jnp.zeros((SEG, D), F32)
        rbuf[...] = jnp.full((SEG, 128), -jnp.inf, F32)

        NC2 = NCH // 2

        def relayout(dst, c, slot):
            for b in range(2 * DC // 16):
                for j in range(HP):
                    ev = stage[slot, pl.ds((b * 16) * HP + j, 8, stride=H), :]
                    od = stage[slot, pl.ds((b * 16 + 1) * HP + j, 8, stride=H), :]
                    lo = (ev & jnp.uint32(0xFFFF)) | (od << 16)
                    hi = (ev >> 16) | (od & jnp.uint32(0xFFFF0000))
                    r0 = pl.multiple_of(c * DC + b * 8, 8)
                    gi, hi_ = divmod(2 * j, G)
                    dst[gi, pl.ds(r0, 8), hi_ * E:(hi_ + 1) * E] = lo
                    dst[gi, pl.ds(r0, 8), (hi_ + 1) * E:(hi_ + 2) * E] = hi

        def body_q(c, carry):
            slot = c % NSLOT
            nslot = (c + PF) % NSLOT
            cp(0, c, slot).wait()

            @pl.when(c + PF < NC2)
            def _():
                cp(0, c + PF, nslot).start()

            @pl.when(c + PF >= NC2)
            def _():
                cp(1, c + PF - NC2, nslot).start()
            relayout(wq, c, slot)
            return carry
        lax.fori_loop(0, NC2, body_q, 0)

        def body_kv(i, carry):
            n = NC2 + i
            slot = n % NSLOT
            nslot = (n + PF) % NSLOT
            c = i % NC2
            pltpu.make_async_copy(stage.at[slot], stage.at[slot], sem_st.at[slot]).wait()

            @pl.when(i + PF < NC2)
            def _():
                cp(1, i + PF, nslot).start()

            @pl.when((i + PF >= NC2) & (i + PF < 2 * NC2))
            def _():
                cp(2, i + PF - NC2, nslot).start()

            @pl.when(i + PF == 2 * NC2)
            def _():
                cp_wo.start()
            relayout(wkv.at[i // NC2], c, slot)
            qpre[i] = _mm(hpre[...], pltpu.bitcast(wq[i], BF16))
            return carry
        assert 2 * NC2 == NG
        lax.fori_loop(0, NG, body_kv, 0)

        def body_kp(i, carry):
            kpre[i] = _mm(hpre[...], pltpu.bitcast(wkv[0, i], BF16))
            return carry
        lax.fori_loop(0, NKP, body_kp, 0)
        cp_wo.wait()
        cp_modB.start()
        cp_x1.start()
        cp_wg.start()
        cp_wu.start()
        cp_wd.start()

        row = lax.broadcasted_iota(jnp.int32, (L, L), 0)
        col = lax.broadcasted_iota(jnp.int32, (L, L), 1)
        mask = (row < M) | (row >= col)
        lane = lax.broadcasted_iota(jnp.int32, (SEG, 128), 1)

        def out_copy2(seg):
            r0 = pl.multiple_of(seg * SEG, 2 * SEG)
            return pltpu.make_async_copy(ostage.at[pl.ds(r0, 2 * SEG)], out_hbm.at[pl.ds(r0, 2 * SEG)], sem_o.at[0])

        def epilogue(seg, o, valid):
            r0 = pl.multiple_of(seg * SEG, SEG)
            xv = xs[pl.ds(r0, SEG), :].astype(F32)
            x1 = _rb(xv + mod_row(2) * o)
            x1s[pl.ds(r0, SEG), :] = x1
            h2 = _rb(_ln(x1) * (1.0 + mod_row(4)) + mod_row(3))
            r = _rb(jnp.sum(h2 * wr_ref[...].astype(F32), axis=-1, keepdims=True))
            rbuf[...] = jnp.where(lane == jnp.where(valid, seg, -1), r, rbuf[...])
            res = x1 + mod_row(5) * h2
            ostage[pl.ds(r0, SEG), :] = res.astype(BF16)
            return r

        def step(s, mem, cur, oslot_w, oslot_r):
            nxt = 1 - cur
            hh = jnp.concatenate([mem, hbuf[cur]], axis=0)
            st = {}
            pr0 = pl.multiple_of(s * PR, PR)

            def Q(g):
                qs = _mm_q(hh[0:L - PR], pltpu.bitcast(wq[g], BF16))
                st['q', g] = jnp.concatenate([qs, qpre[g, pl.ds(pr0, PR), :]], axis=0)

            def K(g):
                if g < NKP:
                    ks = _mm_k(hh[0:L - PR], pltpu.bitcast(wkv[0, g], BF16))
                    st['k', g] = jnp.concatenate([ks, kpre[g, pl.ds(pr0, PR), :]], axis=0).astype(BF16)
                else:
                    st['k', g] = _mm_k(hh, pltpu.bitcast(wkv[0, g], BF16)).astype(BF16)

            def V(g):
                st['v', g] = _mm_v(hh, pltpu.bitcast(wkv[1, g], BF16)).astype(BF16)

            def SC(g):
                q, k = st['q', g], st['k', g]
                st['s', g] = [_mm_nt(q[:, hd * E:(hd + 1) * E], k[:, hd * E:(hd + 1) * E]) for hd in range(G)]

            def PV(g):
                v = st['v', g]
                os_ = []
                for hd in range(G):
                    sc = jnp.where(mask, st['s', g][hd] * scale, -1e9)
                    mx = jnp.max(sc, axis=-1, keepdims=True)
                    e = jnp.exp(sc - mx)
                    p = e * _recip(jnp.sum(e, axis=-1, keepdims=True))
                    os_.append(_mm_pv(p, v[:, hd * E:(hd + 1) * E]))
                st['o', g] = jnp.concatenate(os_, axis=1)

            def WO(g):
                part = (_mm_o if g % 2 else _mm_o2)(st['o', g], pltpu.bitcast(wo[g * G * (E // 2):(g + 1) * G * (E // 2), :], BF16))
                st['acc'] = part if 'acc' not in st else st['acc'] + part

            def WOH(g, h):
                cs = slice(h * (D // 2), (h + 1) * (D // 2))
                part = _mm_o2(st['o', g], pltpu.bitcast(wo[g * G * (E // 2):(g + 1) * G * (E // 2), cs], BF16))
                st['acch', h] = part

            Q(0); K(0); V(0)
            for g in range(NG - 1):
                SC(g); Q(g + 1); K(g + 1); PV(g); V(g + 1)
                if g >= 2:
                    WO(g - 2)
                if g == 0:
                    hn = ln1(jnp.minimum(s + 1, NSEG - 1))
                    hbuf[nxt] = hn
                if g == 2:
                    v3 = st['v', 3]
                    st['v', 3] = jnp.concatenate([v3[0:8], jnp.where(s < 0, hn[:, 0:G * E].astype(BF16), v3[8:L])], axis=0)
                if g == 3:
                    dep = epilogue(jnp.maximum(s - LAG, 0), obuf[oslot_r], s >= LAG)
                if g == 6:
                    q5 = st['q', 7]
                    st['q', 7] = jnp.concatenate([q5[0:8], jnp.where(s < 0, jnp.broadcast_to(dep, (SEG, G * E)), q5[8:L])], axis=0)
            g = NG - 1
            SC(g); WO(g - 2); WOH(g - 1, 0); PV(g); WOH(g - 1, 1); WO(g)
            acc = st['acc'] + jnp.concatenate([st['acch', 0], st['acch', 1]], axis=1)
            obuf[oslot_w] = acc[M:L]
            return acc[0:M]

        def pair(p, mem):
            @pl.when(p == 1)
            def _():
                cp_modB.wait()
                mods[:, 2 * D:6 * D] = _rb(_mm(sc8, pltpu.bitcast(wmodB[...], BF16)))
                cp_x1.wait()

            @pl.when(p > 1)
            def _():
                out_copy2(2 * p - 4).start()
            base = (p % 2) * 2
            mem = step(2 * p, mem, 0, base, 2 - base)
            mem = step(2 * p + 1, mem, 1, base + 1, 3 - base)
            return mem
        lax.fori_loop(0, NSEG // 2, pair, mem0_ref[...].astype(F32))
        out_copy2(NSEG - 4).start()
        epilogue(NSEG - 2, obuf[2], True)
        epilogue(NSEG - 1, obuf[3], True)
        out_copy2(NSEG - 2).start()

        rv = rbuf[...]
        ridx = lane * SEG + lax.broadcasted_iota(jnp.int32, (SEG, 128), 0)

        def allmax(a):
            return jnp.max(jnp.max(a, axis=1, keepdims=True), axis=0, keepdims=True)

        def allmin(a):
            return jnp.min(jnp.min(a, axis=1, keepdims=True), axis=0, keepdims=True)
        m1 = allmax(rv)
        i1 = allmin(jnp.where(rv == m1, ridx, S))
        rv2 = jnp.where(ridx == i1, -jnp.inf, rv)
        m2 = allmax(rv2)
        i2 = allmin(jnp.where(rv2 == m2, ridx, S))
        i1s = jnp.clip(i1[0, 0], 0, S - 1)
        i2s = jnp.clip(i2[0, 0], 0, S - 1)
        xsel[...] = jnp.zeros((8, D), F32)
        xsel[0:1, :] = x1s[pl.ds(i1s, 1), :]
        xsel[1:2, :] = x1s[pl.ds(i2s, 1), :]
        x1sel = xsel[...]
        h2 = _rb(_ln(x1sel) * (1.0 + mod_row(4)) + mod_row(3))
        cp_wg.wait()
        gte = _rb(_mm(h2, pltpu.bitcast(wg[...], BF16)))
        cp_wu.wait()
        up = _rb(_mm(h2, pltpu.bitcast(wu[...], BF16)))
        act = _rb(gte * jax.nn.sigmoid(gte)) * up
        cp_wd.wait()
        y = _rb(_mm(act, pltpu.bitcast(wd[...], BF16)))
        rid8 = lax.broadcasted_iota(jnp.int32, (8, D), 0)
        rsel = jnp.where(rid8 == 0, jnp.broadcast_to(m1, (8, D)), jnp.broadcast_to(m2, (8, D)))
        y = _rb(y * _rb(jax.nn.sigmoid(rsel)))
        fin = x1sel + _rb(mod_row(5) * _rb(h2 + y))
        pltpu.make_async_copy(ostage, out_hbm, sem_o.at[0]).wait()
        bs = []
        for t, ii in ((0, i1s), (1, i2s)):
            b0 = pl.multiple_of((ii // 16) * 16, 16)
            blk = ostage[pl.ds(b0, 16), :].astype(F32)
            rid = lax.broadcasted_iota(jnp.int32, (16, D), 0) + b0
            new = jnp.where(rid == ii, jnp.broadcast_to(fin[t:t + 1, :], (16, D)), blk)
            ostage[pl.ds(b0, 16), :] = new.astype(BF16)
            bs.append(b0)
        for t in range(2):
            cpo = pltpu.make_async_copy(ostage.at[pl.ds(bs[t], 16)], out_hbm.at[pl.ds(bs[t], 16)], sem_o.at[1])
            cpo.start()
            cpo.wait()

    scratch = [
        pltpu.VMEM((NG, D // 2, GE), U32), pltpu.VMEM((2, NG, D // 2, GE), U32),
        pltpu.VMEM((HE // 2, D), U32),
        pltpu.VMEM((D // 2, FF), U32), pltpu.VMEM((D // 2, FF), U32), pltpu.VMEM((FF // 2, D), U32),
        pltpu.VMEM((D // 2, 2 * D), U32), pltpu.VMEM((D // 2, 4 * D), U32),
        pltpu.VMEM((NSLOT, 2 * DC * HP, E), U32),
        pltpu.VMEM((S, D), BF16),
        pltpu.VMEM((NSEG, PR, D), BF16),
        pltpu.VMEM((NSEG * PR, D), F32),
        pltpu.VMEM((NG, NSEG * PR, GE), F32),
        pltpu.VMEM((max(NKP, 1), NSEG * PR, GE), F32),
        pltpu.VMEM((8, 6 * D), F32),
        pltpu.VMEM((2, SEG, D), F32),
        pltpu.VMEM((4, SEG, D), F32),
        pltpu.VMEM((S, D), F32),
        pltpu.VMEM((SEG, 128), F32),
        pltpu.VMEM((S, D), BF16),
        pltpu.VMEM((8, D), F32),
        pltpu.SemaphoreType.DMA((NSLOT,)),
        pltpu.SemaphoreType.DMA((9,)),
        pltpu.SemaphoreType.DMA((2,)),
    ]
    return kernel, scratch


@functools.partial(jax.jit, static_argnames=("A_seg_len",))
def pallas_adaLN_cond__memory_aug_recurrent_mem_tr__moe_arch_mod__prompt_kernel(
        A_x, A_mem0, A_Wq, A_Wk, A_Wv, A_Wo, A_seg_len, B_x, B_w_r, B_w_gate, B_w_up, B_w_down, c, w_mod):
    B, S, D = A_x.shape
    _, H, E = A_Wq.shape
    M = A_mem0.shape[1]
    FF = B_w_gate.shape[1]
    assert B == 1
    kernel, scratch = make_kernel(S, D, H, E, M, int(A_seg_len), FF, 4)
    hbm = pl.BlockSpec(memory_space=pl.ANY)
    vm = pl.BlockSpec(memory_space=pltpu.VMEM)
    out = pl.pallas_call(
        kernel,
        out_shape=jax.ShapeDtypeStruct((S, D), A_x.dtype),
        in_specs=[hbm, hbm, vm, hbm, hbm, hbm, hbm, vm, hbm, hbm, hbm, vm, hbm],
        out_specs=hbm,
        scratch_shapes=scratch,
        compiler_params=pltpu.CompilerParams(vmem_limit_bytes=120 * 2**20),
    )(A_x.reshape(S, D), A_x.reshape(S // int(A_seg_len), int(A_seg_len), D), A_mem0.reshape(M, D), A_Wq.reshape(D * H, E), A_Wk.reshape(D * H, E),
      A_Wv.reshape(D * H, E), A_Wo.reshape(H * E, D), B_w_r.reshape(1, D), B_w_gate, B_w_up, B_w_down, c, w_mod)
    return out.reshape(B, S, D)
```

```python
import functools
import jax
import jax.numpy as jnp
from jax import lax
import jax.experimental.pallas as pl
import jax.experimental.pallas.tpu as pltpu

F32 = jnp.float32
BF16 = jnp.bfloat16
U32 = jnp.uint32
KPRE = 3
U = 4


def _mm(a, b):
    return lax.dot_general(a, b, (((1,), (0,)), ((), ())), preferred_element_type=F32)


def _mm_q(a, b):
    return lax.dot_general(a, b, (((1,), (0,)), ((), ())), preferred_element_type=F32)
def _mm_k(a, b):
    return lax.dot_general(a, b, (((1,), (0,)), ((), ())), preferred_element_type=F32)
def _mm_v(a, b):
    return lax.dot_general(a, b, (((1,), (0,)), ((), ())), preferred_element_type=F32)
def _mm_pv(a, b):
    return lax.dot_general(a, b, (((1,), (0,)), ((), ())), preferred_element_type=F32)
def _mm_o(a, b):
    return lax.dot_general(a, b, (((1,), (0,)), ((), ())), preferred_element_type=F32)
def _mm_o2(a, b):
    return lax.dot_general(a, b, (((1,), (0,)), ((), ())), preferred_element_type=F32)


def _mm_nt(a, b):
    return lax.dot_general(a, b, (((1,), (1,)), ((), ())), preferred_element_type=F32)


def _ln(x, eps=1e-5):
    m = jnp.mean(x, axis=-1, keepdims=True)
    d = x - m
    v = jnp.mean(d * d, axis=-1, keepdims=True)
    return d * lax.rsqrt(v + eps)


def _recip(s):
    r = pl.reciprocal(s, approx=True)
    return r * (2.0 - s * r)


def _rb(x):
    return x.astype(BF16).astype(F32)


def make_kernel(S, D, H, E, M, SEG, FF, G):
    NSEG = S // SEG
    L = M + SEG
    HE = H * E
    DC = 128
    NCH = D // DC
    NSLOT = 3
    PF = NSLOT - 1
    PR = 8
    NG = H // G
    GE = G * E
    NKP = KPRE
    XS0 = U + 2
    LAG = U
    scale = float(E) ** -0.5
    HP = H // 2

    def kernel(x_hbm, x3_hbm, mem0_ref, wq_hbm, wk_hbm, wv_hbm, wo_hbm, wr_ref, wg_hbm, wu_hbm, wd_hbm,
               c_ref, wmod_hbm, out_hbm,
               wq, wkv, wo, wg, wu, wd, wmodA, wmodB, stage, xs, xpre, hpre, qpre, kpre, mods, hbuf, obuf, x1s, rbuf, ostage, xsel, wr_row,
               sem_st, sem_w, sem_o):
        wmod_u = wmod_hbm.bitcast(U32)
        cp_modA = pltpu.make_async_copy(wmod_u.at[:, pl.ds(0, 2 * D)], wmodA, sem_w.at[0])
        cp_modB = pltpu.make_async_copy(wmod_u.at[:, pl.ds(2 * D, 4 * D)], wmodB, sem_w.at[1])
        cp_x0 = pltpu.make_async_copy(x_hbm.at[pl.ds(0, XS0 * SEG)], xs.at[pl.ds(0, XS0 * SEG)], sem_w.at[2])
        cp_x1 = pltpu.make_async_copy(x_hbm.at[pl.ds(XS0 * SEG, S - XS0 * SEG)],
                                      xs.at[pl.ds(XS0 * SEG, S - XS0 * SEG)], sem_w.at[3])
        cp_wo = pltpu.make_async_copy(wo_hbm.bitcast(U32), wo, sem_w.at[4])
        cp_wg = pltpu.make_async_copy(wg_hbm.bitcast(U32), wg, sem_w.at[5])
        cp_wu = pltpu.make_async_copy(wu_hbm.bitcast(U32), wu, sem_w.at[6])
        cp_wd = pltpu.make_async_copy(wd_hbm.bitcast(U32), wd, sem_w.at[7])
        srcs = [wq_hbm.bitcast(U32), wk_hbm.bitcast(U32), wv_hbm.bitcast(U32)]
        cp_xp = pltpu.make_async_copy(x3_hbm.at[:, pl.ds(SEG - PR, PR), :], xpre, sem_w.at[8])

        def cp(w, c, slot):
            return pltpu.make_async_copy(srcs[w].at[pl.ds(c * 2 * DC * HP, 2 * DC * HP)], stage.at[slot], sem_st.at[slot])

        wr_row[...] = wr_ref[...].astype(F32).reshape(1, D)
        cp_modA.start()
        cp_xp.start()
        cp_x0.start()
        for n in range(PF):
            cp(0, n, n).start()

        cc = c_ref[...].astype(F32)
        sc8 = jnp.broadcast_to(cc * jax.nn.sigmoid(cc), (8, D))
        mods[:, 2 * D:6 * D] = jnp.zeros((8, 4 * D), F32)
        cp_modA.wait()
        mods[:, 0:2 * D] = _rb(_mm(sc8, pltpu.bitcast(wmodA[...], BF16)))

        def mod_row(i):
            return mods[0:1, i * D:(i + 1) * D]

        def ln1(seg):
            xv = xs[pl.ds(pl.multiple_of(seg * SEG, SEG), SEG), :].astype(F32)
            return _ln(xv) * (1.0 + mod_row(1)) + mod_row(0)

        cp_xp.wait()
        xp = xpre[...].astype(F32).reshape(NSEG * PR, D)
        hpre[...] = _ln(xp) * (1.0 + mod_row(1)) + mod_row(0)
        cp_x0.wait()
        hbuf[0] = ln1(0)
        for i in range(2 * U):
            obuf[i] = jnp.zeros((SEG, D), F32)
        rbuf[...] = jnp.full((SEG, 128), -jnp.inf, F32)

        NC2 = NCH // 2

        def relayout(dst, c, slot):
            for b in range(2 * DC // 16):
                for j in range(HP):
                    ev = stage[slot, pl.ds((b * 16) * HP + j, 8, stride=H), :]
                    od = stage[slot, pl.ds((b * 16 + 1) * HP + j, 8, stride=H), :]
                    lo = (ev & jnp.uint32(0xFFFF)) | (od << 16)
                    hi = (ev >> 16) | (od & jnp.uint32(0xFFFF0000))
                    r0 = pl.multiple_of(c * DC + b * 8, 8)
                    gi, hi_ = divmod(2 * j, G)
                    dst[gi, pl.ds(r0, 8), hi_ * E:(hi_ + 1) * E] = lo
                    dst[gi, pl.ds(r0, 8), (hi_ + 1) * E:(hi_ + 2) * E] = hi

        def body_q(c, carry):
            slot = c % NSLOT
            nslot = (c + PF) % NSLOT
            cp(0, c, slot).wait()

            @pl.when(c + PF < NC2)
            def _():
                cp(0, c + PF, nslot).start()

            @pl.when(c + PF >= NC2)
            def _():
                cp(1, c + PF - NC2, nslot).start()
            relayout(wq, c, slot)
            return carry
        lax.fori_loop(0, NC2, body_q, 0)

        def body_kv(i, carry):
            n = NC2 + i
            slot = n % NSLOT
            nslot = (n + PF) % NSLOT
            c = i % NC2
            pltpu.make_async_copy(stage.at[slot], stage.at[slot], sem_st.at[slot]).wait()

            @pl.when(i + PF < NC2)
            def _():
                cp(1, i + PF, nslot).start()

            @pl.when((i + PF >= NC2) & (i + PF < 2 * NC2))
            def _():
                cp(2, i + PF - NC2, nslot).start()

            @pl.when(i + PF == 2 * NC2)
            def _():
                cp_wo.start()
            relayout(wkv.at[i // NC2], c, slot)
            qpre[i] = _mm(hpre[...], pltpu.bitcast(wq[i], BF16))
            return carry
        assert 2 * NC2 == NG
        lax.fori_loop(0, NG, body_kv, 0)

        def body_kp(i, carry):
            kpre[i] = _mm(hpre[...], pltpu.bitcast(wkv[0, i], BF16))
            return carry
        lax.fori_loop(0, NKP, body_kp, 0)
        cp_wo.wait()
        cp_modB.start()
        cp_x1.start()
        cp_wg.start()
        cp_wu.start()
        cp_wd.start()

        row = lax.broadcasted_iota(jnp.int32, (L, L), 0)
        col = lax.broadcasted_iota(jnp.int32, (L, L), 1)
        mask = (row < M) | (row >= col)
        lane = lax.broadcasted_iota(jnp.int32, (SEG, 128), 1)

        def out_copy(seg, n):
            r0 = pl.multiple_of(seg * SEG, n * SEG) if not isinstance(seg, int) else seg * SEG
            return pltpu.make_async_copy(ostage.at[pl.ds(r0, n * SEG)], out_hbm.at[pl.ds(r0, n * SEG)], sem_o.at[0])

        def epilogue(seg, o, valid):
            r0 = pl.multiple_of(seg * SEG, SEG)
            xv = xs[pl.ds(r0, SEG), :].astype(F32)
            x1 = _rb(xv + mod_row(2) * o)
            x1s[pl.ds(r0, SEG), :] = x1
            h2 = _rb(_ln(x1) * (1.0 + mod_row(4)) + mod_row(3))
            r = _rb(jnp.sum(h2 * wr_row[...], axis=-1, keepdims=True))
            rbuf[...] = jnp.where(lane == jnp.where(valid, seg, -1), r, rbuf[...])
            res = x1 + mod_row(5) * h2
            ostage[pl.ds(r0, SEG), :] = res.astype(BF16)
            return r

        def step(s, mem, cur, oslot_w, oslot_r):
            nxt = 1 - cur
            hh = jnp.concatenate([mem, hbuf[cur]], axis=0)
            st = {}
            pr0 = pl.multiple_of(s * PR, PR)

            def Q(g):
                qs = _mm_q(hh[0:L - PR], pltpu.bitcast(wq[g], BF16))
                st['q', g] = jnp.concatenate([qs, qpre[g, pl.ds(pr0, PR), :]], axis=0)

            def K(g):
                if g < NKP:
                    ks = _mm_k(hh[0:L - PR], pltpu.bitcast(wkv[0, g], BF16))
                    st['k', g] = jnp.concatenate([ks, kpre[g, pl.ds(pr0, PR), :]], axis=0).astype(BF16)
                else:
                    st['k', g] = _mm_k(hh, pltpu.bitcast(wkv[0, g], BF16)).astype(BF16)

            def V(g):
                st['v', g] = _mm_v(hh, pltpu.bitcast(wkv[1, g], BF16)).astype(BF16)

            def SC(g):
                q, k = st['q', g], st['k', g]
                st['s', g] = [_mm_nt(q[:, hd * E:(hd + 1) * E], k[:, hd * E:(hd + 1) * E]) for hd in range(G)]

            def PV(g):
                v = st['v', g]
                os_ = []
                for hd in range(G):
                    sc = jnp.where(mask, st['s', g][hd] * scale, -1e9)
                    mx = jnp.max(sc, axis=-1, keepdims=True)
                    e = jnp.exp(sc - mx)
                    p = e * _recip(jnp.sum(e, axis=-1, keepdims=True))
                    os_.append(_mm_pv(p, v[:, hd * E:(hd + 1) * E]))
                st['o', g] = jnp.concatenate(os_, axis=1)

            def WO(g):
                part = (_mm_o if g % 2 else _mm_o2)(st['o', g], pltpu.bitcast(wo[g * G * (E // 2):(g + 1) * G * (E // 2), :], BF16))
                st['acc'] = part if 'acc' not in st else st['acc'] + part

            def WOH(g, h):
                cs = slice(h * (D // 2), (h + 1) * (D // 2))
                part = _mm_o2(st['o', g], pltpu.bitcast(wo[g * G * (E // 2):(g + 1) * G * (E // 2), cs], BF16))
                st['acch', h] = part

            Q(0); K(0); V(0)
            for g in range(NG - 1):
                SC(g); Q(g + 1); K(g + 1); PV(g); V(g + 1)
                if g >= 2:
                    WO(g - 2)
                if g == 0:
                    hn = ln1(jnp.minimum(s + 1, NSEG - 1))
                    hbuf[nxt] = hn
                if g == 2:
                    v3 = st['v', 3]
                    st['v', 3] = jnp.concatenate([v3[0:8], jnp.where(s < 0, hn[:, 0:G * E].astype(BF16), v3[8:L])], axis=0)
                if g == 2:
                    dep = epilogue(jnp.maximum(s - LAG, 0), obuf[oslot_r], s >= LAG)
                if g == 6:
                    q5 = st['q', 7]
                    st['q', 7] = jnp.concatenate([q5[0:8], jnp.where(s < 0, jnp.broadcast_to(dep, (SEG, G * E)), q5[8:L])], axis=0)
            g = NG - 1
            SC(g); WO(g - 2); WOH(g - 1, 0); PV(g); WOH(g - 1, 1); WO(g)
            acc = st['acc'] + jnp.concatenate([st['acch', 0], st['acch', 1]], axis=1)
            obuf[oslot_w] = acc[M:L]
            return acc[0:M]

        def block(p, mem):
            @pl.when(p == 1)
            def _():
                cp_modB.wait()
                mods[:, 2 * D:6 * D] = _rb(_mm(sc8, pltpu.bitcast(wmodB[...], BF16)))
                cp_x1.wait()

            @pl.when(p > 1)
            def _():
                out_copy(U * (p - 2), U).start()
            base = (p % 2) * U
            for i in range(U):
                mem = step(U * p + i, mem, i % 2, base + i, U - base + i)
            return mem
        NP = NSEG // U
        lax.fori_loop(0, NP, block, mem0_ref[...].astype(F32))
        out_copy(U * (NP - 2), U).start()
        for i in range(U):
            epilogue(U * (NP - 1) + i, obuf[((NP - 1) % 2) * U + i], True)
        out_copy(U * (NP - 1), U).start()

        rv = rbuf[...]
        ridx = lane * SEG + lax.broadcasted_iota(jnp.int32, (SEG, 128), 0)

        def allmax(a):
            return jnp.max(jnp.max(a, axis=1, keepdims=True), axis=0, keepdims=True)

        def allmin(a):
            return jnp.min(jnp.min(a, axis=1, keepdims=True), axis=0, keepdims=True)
        m1 = allmax(rv)
        i1 = allmin(jnp.where(rv == m1, ridx, S))
        rv2 = jnp.where(ridx == i1, -jnp.inf, rv)
        m2 = allmax(rv2)
        i2 = allmin(jnp.where(rv2 == m2, ridx, S))
        i1s = jnp.clip(i1[0, 0], 0, S - 1)
        i2s = jnp.clip(i2[0, 0], 0, S - 1)
        xsel[...] = jnp.zeros((8, D), F32)
        xsel[0:1, :] = x1s[pl.ds(i1s, 1), :]
        xsel[1:2, :] = x1s[pl.ds(i2s, 1), :]
        x1sel = xsel[...]
        h2 = _rb(_ln(x1sel) * (1.0 + mod_row(4)) + mod_row(3))
        cp_wg.wait()
        gte = _rb(_mm(h2, pltpu.bitcast(wg[...], BF16)))
        cp_wu.wait()
        up = _rb(_mm(h2, pltpu.bitcast(wu[...], BF16)))
        act = _rb(gte * jax.nn.sigmoid(gte)) * up
        cp_wd.wait()
        y = _rb(_mm(act, pltpu.bitcast(wd[...], BF16)))
        rid8 = lax.broadcasted_iota(jnp.int32, (8, D), 0)
        rsel = jnp.where(rid8 == 0, jnp.broadcast_to(m1, (8, D)), jnp.broadcast_to(m2, (8, D)))
        y = _rb(y * _rb(jax.nn.sigmoid(rsel)))
        fin = x1sel + _rb(mod_row(5) * _rb(h2 + y))
        pltpu.make_async_copy(ostage, out_hbm, sem_o.at[0]).wait()
        bs = []
        for t, ii in ((0, i1s), (1, i2s)):
            b0 = pl.multiple_of((ii // 16) * 16, 16)
            blk = ostage[pl.ds(b0, 16), :].astype(F32)
            rid = lax.broadcasted_iota(jnp.int32, (16, D), 0) + b0
            new = jnp.where(rid == ii, jnp.broadcast_to(fin[t:t + 1, :], (16, D)), blk)
            ostage[pl.ds(b0, 16), :] = new.astype(BF16)
            bs.append(b0)
        def patch_copy(t):
            return pltpu.make_async_copy(ostage.at[pl.ds(bs[t], 16)], out_hbm.at[pl.ds(bs[t], 16)], sem_o.at[1 + t])
        patch_copy(0).start()

        @pl.when(bs[0] != bs[1])
        def _():
            patch_copy(1).start()
            patch_copy(1).wait()
        patch_copy(0).wait()

    scratch = [
        pltpu.VMEM((NG, D // 2, GE), U32), pltpu.VMEM((2, NG, D // 2, GE), U32),
        pltpu.VMEM((HE // 2, D), U32),
        pltpu.VMEM((D // 2, FF), U32), pltpu.VMEM((D // 2, FF), U32), pltpu.VMEM((FF // 2, D), U32),
        pltpu.VMEM((D // 2, 2 * D), U32), pltpu.VMEM((D // 2, 4 * D), U32),
        pltpu.VMEM((NSLOT, 2 * DC * HP, E), U32),
        pltpu.VMEM((S, D), BF16),
        pltpu.VMEM((NSEG, PR, D), BF16),
        pltpu.VMEM((NSEG * PR, D), F32),
        pltpu.VMEM((NG, NSEG * PR, GE), F32),
        pltpu.VMEM((max(NKP, 1), NSEG * PR, GE), F32),
        pltpu.VMEM((8, 6 * D), F32),
        pltpu.VMEM((2, SEG, D), F32),
        pltpu.VMEM((2 * U, SEG, D), F32),
        pltpu.VMEM((S, D), F32),
        pltpu.VMEM((SEG, 128), F32),
        pltpu.VMEM((S, D), BF16),
        pltpu.VMEM((8, D), F32),
        pltpu.VMEM((1, D), F32),
        pltpu.SemaphoreType.DMA((NSLOT,)),
        pltpu.SemaphoreType.DMA((9,)),
        pltpu.SemaphoreType.DMA((3,)),
    ]
    return kernel, scratch


@functools.partial(jax.jit, static_argnames=("A_seg_len",))
def pallas_adaLN_cond__memory_aug_recurrent_mem_tr__moe_arch_mod__prompt_kernel(
        A_x, A_mem0, A_Wq, A_Wk, A_Wv, A_Wo, A_seg_len, B_x, B_w_r, B_w_gate, B_w_up, B_w_down, c, w_mod):
    B, S, D = A_x.shape
    _, H, E = A_Wq.shape
    M = A_mem0.shape[1]
    FF = B_w_gate.shape[1]
    assert B == 1
    kernel, scratch = make_kernel(S, D, H, E, M, int(A_seg_len), FF, 4)
    hbm = pl.BlockSpec(memory_space=pl.ANY)
    vm = pl.BlockSpec(memory_space=pltpu.VMEM)
    out = pl.pallas_call(
        kernel,
        out_shape=jax.ShapeDtypeStruct((S, D), A_x.dtype),
        in_specs=[hbm, hbm, vm, hbm, hbm, hbm, hbm, vm, hbm, hbm, hbm, vm, hbm],
        out_specs=hbm,
        scratch_shapes=scratch,
        compiler_params=pltpu.CompilerParams(vmem_limit_bytes=120 * 2**20),
    )(A_x.reshape(S, D), A_x.reshape(S // int(A_seg_len), int(A_seg_len), D), A_mem0.reshape(M, D), A_Wq.reshape(D * H, E), A_Wk.reshape(D * H, E),
      A_Wv.reshape(D * H, E), A_Wo.reshape(H * E, D), B_w_r, B_w_gate, B_w_up, B_w_down, c, w_mod)
    return out.reshape(B, S, D)
```
